```python
import os as _os
_os.environ.setdefault("JAX_PLATFORMS", "cpu")
import jax
import jax.numpy as jnp

def _softmax(x, axis=-1):
    return jax.nn.softmax(x, axis=axis)
def _gelu(x):
    return jax.nn.gelu(x, approximate=True)
def _silu(x):
    return jax.nn.silu(x)
def _sigmoid(x):
    return jax.nn.sigmoid(x)
def _layernorm(x, axis=-1, eps=1e-5):
    m = jnp.mean(x, axis=axis, keepdims=True)
    v = jnp.var(x, axis=axis, keepdims=True)
    return (x - m) / jnp.sqrt(v + eps)
def _scatter_add(tgt, idx, src, axis=0):
    return tgt.at[idx].add(src)
def _segment_sum(src, seg, n):
    return jax.ops.segment_sum(src, seg, n)
class _Rng:
    def __init__(self, key):
        self._k = key
    def _next(self):
        self._k, sub = jax.random.split(self._k)
        return sub
    def normal(self, shape):
        return jax.random.normal(self._next(), shape, dtype=jnp.bfloat16)
    def randint(self, lo, hi, shape):
        return jax.random.randint(self._next(), shape, lo, hi, dtype=jnp.int32)
    def uniform(self, shape, lo=0.0, hi=1.0):
        return jax.random.uniform(self._next(), shape, jnp.bfloat16, lo, hi)
    def permutation(self, n):
        return jax.random.permutation(self._next(), n)


kernel_name = 'standalone__gqa_block_cached__near_ridge'

def setup_inputs():
    _rng = _Rng(jax.random.key(int.from_bytes(__import__("os").urandom(4), "little")))
    _w = (lambda a: (lambda t: t.astype(jnp.bfloat16) if jnp.issubdtype(t.dtype, jnp.floating) else t)(jnp.asarray(a)))
    B, Sq, D = 8, 96, 640
    Hq, Hkv, Sk, Dh = 32, 32, 512, 128
    assert Hq % Hkv == 0, (Hq, Hkv)
    return {
        "x": _w((lambda *s: _rng.normal(s) * 0.2)(B, Sq, D)),
        "k_cache": _w((lambda *s: _rng.normal(s) * 3.2)(B, Hkv, Sk, Dh)),
        "v_cache": _w((lambda *s: _rng.normal(s) * 0.05)(B, Hkv, Sk, Dh)),
        "wq": _w((lambda *s: _rng.normal(s) * 0.2)(D, Hq * Dh) * (D ** -0.5)),
        "wo": _w((lambda *s: _rng.normal(s) * 0.05)(Hq * Dh, D) * ((Hq * Dh) ** -0.5)),
    }

def reference(x, k_cache, v_cache, wq, wo):
    B, Sq, D = x.shape
    Hq, Dh = 32, 128
    Hkv = k_cache.shape[1]
    rep = Hq // Hkv
    q = (lambda x, *d: x.transpose(*d))((x @ wq).reshape(B, Sq, Hq, Dh), 0, 2, 1, 3)
    k = jnp.repeat(k_cache, rep, axis=1)
    v = jnp.repeat(v_cache, rep, axis=1)
    scores = jnp.einsum("bhqd,bhkd->bhqk", q, k) * (Dh ** -0.5)
    p = _softmax(scores, axis=-1)
    o = jnp.einsum("bhqk,bhkd->bhqd", p, v)
    return (lambda x, *d: x.transpose(*d))(o, 0, 2, 1, 3).reshape(B, Sq, Hq * Dh) @ wo
```

```python
import math

import jax
import jax.numpy as jnp
import jax.experimental.pallas as pl
import jax.experimental.pallas.tpu as pltpu

_GH = 4
_L = 4


@jax.jit
def pallas_standalone__gqa_block_cached__near_ridge_kernel(
    x: jax.Array,
    k_cache: jax.Array,
    v_cache: jax.Array,
    wq: jax.Array,
    wo: jax.Array,
):
    B, SQ, D = x.shape
    _, HKV, SK, DH = k_cache.shape
    H = wq.shape[1] // DH
    assert HKV == H, "one KV head per query head at these shapes"
    GH, L = _GH, _L
    assert H % GH == 0
    NG = H // GH
    GW = GH * DH
    NS = NG * B
    f32, bf16 = jnp.float32, jnp.bfloat16
    q_scale = float(DH ** -0.5 * math.log2(math.e))

    def kernel(x_hbm, k_hbm, v_hbm, wq_hbm, wo_hbm, out_hbm,
               x_v, k_v, v_v, wq_v, wo_v, q_v, o_v, acc, out_v,
               x_sem, k_sem, v_sem, wq_sem, wo_sem, out_sem):

        def cp_x():
            return pltpu.make_async_copy(x_hbm, x_v, x_sem)

        def cp_wq(g):
            return pltpu.make_async_copy(wq_hbm.at[:, pl.ds(g * GW, GW)], wq_v.at[g], wq_sem.at[g])

        def cp_wo(g):
            return pltpu.make_async_copy(wo_hbm.at[pl.ds(g * GW, GW), :], wo_v.at[g], wo_sem.at[g])

        def cp_k(g, b, slot):
            return pltpu.make_async_copy(k_hbm.at[b, pl.ds(g * GH, GH)], k_v.at[slot], k_sem.at[slot])

        def cp_v(g, b, slot):
            return pltpu.make_async_copy(v_hbm.at[b, pl.ds(g * GH, GH)], v_v.at[slot], v_sem.at[slot])

        def cp_out_head():
            return pltpu.make_async_copy(out_v.at[pl.ds(0, B - 1)], out_hbm.at[pl.ds(0, B - 1)], out_sem.at[0])

        def cp_out_tail():
            return pltpu.make_async_copy(out_v.at[pl.ds(B - 1, 1)], out_hbm.at[pl.ds(B - 1, 1)], out_sem.at[1])

        def start_kv(i, slot):
            cp_k(i // B, i % B, slot).start()
            cp_v(i // B, i % B, slot).start()

        def start_weights(g):
            cp_wo(g).start()
            if isinstance(g, int):
                if g + 1 < NG:
                    cp_wq(g + 1).start()
            else:
                @pl.when(g + 1 < NG)
                def _():
                    cp_wq(g + 1).start()

        def q_proj(g, b, qslot):
            q = jnp.dot(x_v[b], wq_v[g], preferred_element_type=f32)
            q_v[qslot] = (q * q_scale).astype(bf16)

        def scores(qslot, slot, h):
            q = q_v[qslot, :, h * DH:(h + 1) * DH]
            return jax.lax.dot_general(q, k_v[slot, h], (((1,), (1,)), ((), ())), preferred_element_type=f32)

        def softmax(s):
            m = jnp.max(s, axis=-1, keepdims=True)
            e = jnp.exp2(s - m)
            l = jnp.sum(e, axis=-1, keepdims=True)
            r = pl.reciprocal(l, approx=True)
            r = r * (2.0 - l * r)
            return e.astype(bf16), r

        def weighted(slot, h, e, r):
            o = jnp.dot(e, v_v[slot, h], preferred_element_type=f32)
            o_v[:, h * DH:(h + 1) * DH] = (o * r).astype(bf16)

        def o_proj(g, b):
            a = acc[b] + jnp.dot(o_v[...], wo_v[g], preferred_element_type=f32)
            acc[b] = a
            out_v[b] = a.astype(bf16)

        def step(i, carry):
            slot, g, b, qslot = carry
            wrap = b == B - 1
            bn = jnp.where(wrap, 0, b + 1)
            gn = jnp.where(wrap, g + 1, g)
            last = i == NS - 1
            bq = jnp.where(last, b, bn)
            gq = jnp.where(last, g, gn)

            @pl.when(b == 0)
            def _():
                cp_wo(g).wait()

                @pl.when(g + 1 < NG)
                def _():
                    cp_wq(g + 1).wait()

            cp_k(g, b, slot).wait()
            cp_v(g, b, slot).wait()

            @pl.when(last)
            def _():
                cp_out_head().start()

            s0 = scores(qslot, slot, 0)
            s1 = scores(qslot, slot, 1)
            s2 = scores(qslot, slot, 2)
            weighted(slot, 0, *softmax(s0))
            s3 = scores(qslot, slot, 3)
            weighted(slot, 1, *softmax(s1))
            weighted(slot, 2, *softmax(s2))
            q_proj(gq, bq, 1 - qslot)
            weighted(slot, 3, *softmax(s3))
            o_proj(g, b)

            @pl.when(i + L < NS)
            def _():
                i2 = i + L

                @pl.when(i2 % B == 0)
                def _():
                    start_weights(i2 // B)
                start_kv(i2, slot)

            return jnp.where(slot == L - 1, 0, slot + 1), gn, bn, 1 - qslot

        cp_x().start()
        cp_wq(0).start()
        for i in range(L):
            if i % B == 0:
                start_weights(i // B)
            start_kv(i, i)
        acc[...] = jnp.zeros(acc.shape, f32)
        cp_x().wait()
        cp_wq(0).wait()
        q_proj(0, 0, 0)
        jax.lax.fori_loop(0, NS, step, (0, 0, 0, 0))
        cp_out_tail().start()
        cp_out_head().wait()
        cp_out_tail().wait()

    return pl.pallas_call(
        kernel,
        in_specs=[pl.BlockSpec(memory_space=pl.ANY)] * 5,
        out_specs=pl.BlockSpec(memory_space=pl.ANY),
        out_shape=jax.ShapeDtypeStruct((B, SQ, D), x.dtype),
        scratch_shapes=[
            pltpu.VMEM((B, SQ, D), bf16),
            pltpu.VMEM((L, GH, SK, DH), bf16),
            pltpu.VMEM((L, GH, SK, DH), bf16),
            pltpu.VMEM((NG, D, GW), bf16),
            pltpu.VMEM((NG, GW, D), bf16),
            pltpu.VMEM((2, SQ, GW), bf16),
            pltpu.VMEM((SQ, GW), bf16),
            pltpu.VMEM((B, SQ, D), f32),
            pltpu.VMEM((B, SQ, D), bf16),
            pltpu.SemaphoreType.DMA(()),
            pltpu.SemaphoreType.DMA((L,)),
            pltpu.SemaphoreType.DMA((L,)),
            pltpu.SemaphoreType.DMA((NG,)),
            pltpu.SemaphoreType.DMA((NG,)),
            pltpu.SemaphoreType.DMA((2,)),
        ],
        compiler_params=pltpu.CompilerParams(
            vmem_limit_bytes=48 * 1024 * 1024,
            disable_bounds_checks=True,
        ),
    )(x, k_cache, v_cache, wq, wo)
```

```python
import math

import jax
import jax.numpy as jnp
import jax.experimental.pallas as pl
import jax.experimental.pallas.tpu as pltpu

_GH = 4
_L = 4
_STAGED = 3
_STAGE_PER = 2
_X0_ROWS = 48
_WQ0_ROWS = 16
_KV_ROWS = 128
_W_ROWS = 32
_O_ROWS = 16
_K_SPLIT = (8, 0, 3)
_V_SPLIT = (7, 2, 0)
_TAIL = 2


@jax.jit
def pallas_standalone__gqa_block_cached__near_ridge_kernel(
    x: jax.Array,
    k_cache: jax.Array,
    v_cache: jax.Array,
    wq: jax.Array,
    wo: jax.Array,
):
    B, SQ, D = x.shape
    _, HKV, SK, DH = k_cache.shape
    H = wq.shape[1] // DH
    assert HKV == H, "one KV head per query head at these shapes"
    GH, L, STAGED, TAIL = _GH, _L, _STAGED, _TAIL
    assert H % GH == 0 and GH % 2 == 0 and L <= B and STAGED < L
    NG = H // GH
    GW = GH * DH
    assert NG >= 2
    f32, bf16 = jnp.float32, jnp.bfloat16
    q_scale = float(DH ** -0.5 * math.log2(math.e))

    KR, WR, OR = _KV_ROWS, _W_ROWS, _O_ROWS
    assert SK % KR == 0 and D % (2 * WR) == 0 and GW % (2 * WR) == 0 and SQ % OR == 0
    PER_HEAD = SK // KR
    PIECES = (GH // 2) * PER_HEAD
    STAGE_PER = _STAGE_PER
    assert PIECES % STAGE_PER == 0 and STAGED * STAGE_PER <= B
    XR0, WQR0 = _X0_ROWS, _WQ0_ROWS
    assert SQ % XR0 == 0 and D % WQR0 == 0

    def kernel(x_hbm, k_hbm, v_hbm, wq_hbm, wo_hbm, out_hbm,
               x_v, k_v, v_v, wq_v, wo_v, q_v, o_v, acc, out_v,
               x_sem, k_sem, v_sem, wq_sem, wo_sem, out_sem):

        def wait_for(buf, sem):
            pltpu.make_async_copy(buf, buf, sem).wait()

        def start_wq(g, rows=WR):
            n = D // (2 * rows)
            for j in range(n):
                for queue in range(2):
                    r = (queue * n + j) * rows
                    pltpu.make_async_copy(
                        wq_hbm.at[pl.ds(r, rows), pl.ds(g * GW, GW)],
                        wq_v.at[g, pl.ds(r, rows)], wq_sem.at[g]).start(priority=queue)

        def start_wo(g, rows=WR):
            n = GW // (2 * rows)
            for j in range(n):
                for queue in range(2):
                    r = (queue * n + j) * rows
                    pltpu.make_async_copy(
                        wo_hbm.at[pl.ds(g * GW + r, rows), :],
                        wo_v.at[g, pl.ds(r, rows)], wo_sem.at[g]).start(priority=queue)

        def start_kv_piece(src, dst, sem, g, b, slot, head, key0, rows, queue):
            pltpu.make_async_copy(
                src.at[b, g * GH + head, pl.ds(key0, rows)],
                dst.at[slot, head, pl.ds(key0, rows)], sem.at[slot]).start(priority=queue)

        def start_kv(g, b, slot):
            for src, dst, sem, (n_first, rot0, rot1) in ((k_hbm, k_v, k_sem, _K_SPLIT),
                                                         (v_hbm, v_v, v_sem, _V_SPLIT)):
                pieces = list(range(GH * PER_HEAD))
                first, second = pieces[:n_first], pieces[n_first:]
                first = first[rot0:] + first[:rot0]
                second = second[rot1:] + second[:rot1]
                for j in range(max(len(first), len(second))):
                    for queue, lst in enumerate((first, second)):
                        if j < len(lst):
                            start_kv_piece(src, dst, sem, g, b, slot, lst[j] // PER_HEAD,
                                           (lst[j] % PER_HEAD) * KR, KR, queue)

        def wait_kv(slot):
            wait_for(k_v.at[slot], k_sem.at[slot])
            wait_for(v_v.at[slot], v_sem.at[slot])

        def start_out(b0, nb, sem):
            n = 0
            for b in range(b0, b0 + nb):
                for r in range(0, SQ, OR):
                    pltpu.make_async_copy(out_v.at[b, pl.ds(r, OR)], out_hbm.at[b, pl.ds(r, OR)],
                                          sem).start(priority=n % 2)
                    n += 1

        def q_proj(g, b, qslot):
            q = jnp.dot(x_v[b], wq_v[g], preferred_element_type=f32)
            q_v[qslot, b] = (q * q_scale).astype(bf16)

        def scores(qslot, b, slot, h):
            q = q_v[qslot, b, :, h * DH:(h + 1) * DH]
            return jax.lax.dot_general(q, k_v[slot, h], (((1,), (1,)), ((), ())),
                                       preferred_element_type=f32)

        def softmax_pv(slot, h, s):
            m = jnp.max(s, axis=-1, keepdims=True)
            e = jnp.exp2(s - m)
            l = jnp.sum(e, axis=-1, keepdims=True)
            r = pl.reciprocal(l, approx=True)
            r = r * (2.0 - l * r)
            o = jnp.dot(e.astype(bf16), v_v[slot, h], preferred_element_type=f32)
            o_v[:, h * DH:(h + 1) * DH] = (o * r).astype(bf16)

        def o_proj(g, b):
            a = acc[b] + jnp.dot(o_v[...], wo_v[g], preferred_element_type=f32)
            acc[b] = a
            out_v[b] = a.astype(bf16)

        def next_slot(slot):
            return jnp.where(slot == L - 1, 0, slot + 1)

        XP = SQ // XR0
        assert B * XP == GW // WR

        def wq_piece(j, _):
            r = pl.multiple_of(j * WQR0, WQR0)
            pltpu.make_async_copy(wq_hbm.at[pl.ds(r, WQR0), pl.ds(GW, GW)], wq_v.at[1, pl.ds(r, WQR0)],
                                  wq_sem.at[1]).start(priority=1)
            pltpu.make_async_copy(wq_hbm.at[pl.ds(r, WQR0), pl.ds(0, GW)], wq_v.at[0, pl.ds(r, WQR0)],
                                  wq_sem.at[0]).start(priority=0)
            return None

        def x_piece(j, _):
            r = pl.multiple_of(j * WR, WR)
            pltpu.make_async_copy(wo_hbm.at[pl.ds(r, WR), :], wo_v.at[0, pl.ds(r, WR)],
                                  wo_sem.at[0]).start(priority=1)
            b, xr = j // XP, pl.multiple_of((j % XP) * XR0, XR0)
            pltpu.make_async_copy(x_hbm.at[b, pl.ds(xr, XR0)], x_v.at[b, pl.ds(xr, XR0)],
                                  x_sem).start(priority=0)
            return None

        jax.lax.fori_loop(0, D // WQR0, wq_piece, None)
        jax.lax.fori_loop(0, B * XP, x_piece, None)
        for i in range(L - STAGED):
            start_kv(0, i, i)
        acc[...] = jnp.zeros(acc.shape, f32)
        wait_for(x_v, x_sem)
        wait_for(wq_v.at[0], wq_sem.at[0])

        def first_q_proj(b, _):
            @pl.when(b < STAGED * STAGE_PER)
            def _():
                step = L - STAGED + b // STAGE_PER
                part = b % STAGE_PER
                cnt = PIECES // STAGE_PER
                for c in range(cnt):
                    p = part * cnt + c
                    key0 = pl.multiple_of((p % PER_HEAD) * KR, KR)
                    for src, dst, sem in ((k_hbm, k_v, k_sem), (v_hbm, v_v, v_sem)):
                        for queue in range(2):
                            start_kv_piece(src, dst, sem, 0, step, step,
                                           queue * (GH // 2) + p // PER_HEAD, key0, KR, queue)
            q_proj(0, b, 0)
            return None

        jax.lax.fori_loop(0, B, first_q_proj, None)

        def group(g, slot):
            @pl.when(g + 2 < NG)
            def _():
                start_wq(g + 2)
            start_wo(g + 1)
            wait_for(wq_v.at[g + 1], wq_sem.at[g + 1])
            wait_for(wo_v.at[g], wo_sem.at[g])
            qslot = g & 1

            def step(b, slot):
                wait_kv(slot)
                s0 = scores(qslot, b, slot, 0)
                s1 = scores(qslot, b, slot, 1)
                s2 = scores(qslot, b, slot, 2)
                softmax_pv(slot, 0, s0)
                s3 = scores(qslot, b, slot, 3)
                softmax_pv(slot, 1, s1)
                softmax_pv(slot, 2, s2)
                softmax_pv(slot, 3, s3)
                q_proj(g + 1, b, 1 - qslot)
                ahead = b + L
                wrap = (ahead >= B).astype(jnp.int32)
                start_kv(g + wrap, ahead - wrap * B, slot)
                o_proj(g, b)
                return next_slot(slot)

            return jax.lax.fori_loop(0, B, step, slot)

        slot = jax.lax.fori_loop(0, NG - 1, group, 0)

        wait_for(wo_v.at[NG - 1], wo_sem.at[NG - 1])

        def last_step(b, slot):
            qslot = (NG - 1) & 1
            wait_kv(slot)

            @pl.when(b == B - 1)
            def _():
                start_out(0, B - 1, out_sem.at[0])

            s0 = scores(qslot, b, slot, 0)
            s1 = scores(qslot, b, slot, 1)
            s2 = scores(qslot, b, slot, 2)
            softmax_pv(slot, 0, s0)
            s3 = scores(qslot, b, slot, 3)
            softmax_pv(slot, 1, s1)
            softmax_pv(slot, 2, s2)
            softmax_pv(slot, 3, s3)
            o_proj(NG - 1, b)

            @pl.when(b + L + TAIL < B)
            def _():
                start_kv(NG - 1, b + L, slot)

            @pl.when(jnp.logical_and(b + L + TAIL >= B, b + L < B))
            def _():
                for src, dst, sem in ((k_hbm, k_v, k_sem), (v_hbm, v_v, v_sem)):
                    pltpu.make_async_copy(src.at[b + L, pl.ds((NG - 1) * GH, GH)], dst.at[slot],
                                          sem.at[slot]).start(priority=1)

            return next_slot(slot)

        jax.lax.fori_loop(0, B, last_step, slot)
        start_out(B - 1, 1, out_sem.at[1])
        pltpu.make_async_copy(out_v.at[pl.ds(0, B - 1)], out_hbm.at[pl.ds(0, B - 1)],
                              out_sem.at[0]).wait()
        pltpu.make_async_copy(out_v.at[pl.ds(B - 1, 1)], out_hbm.at[pl.ds(B - 1, 1)],
                              out_sem.at[1]).wait()

    assert GH == 4
    return pl.pallas_call(
        kernel,
        in_specs=[pl.BlockSpec(memory_space=pl.ANY)] * 5,
        out_specs=pl.BlockSpec(memory_space=pl.ANY),
        out_shape=jax.ShapeDtypeStruct((B, SQ, D), bf16),
        scratch_shapes=[
            pltpu.VMEM((B, SQ, D), bf16),
            pltpu.VMEM((L, GH, SK, DH), bf16),
            pltpu.VMEM((L, GH, SK, DH), bf16),
            pltpu.VMEM((NG, D, GW), bf16),
            pltpu.VMEM((NG, GW, D), bf16),
            pltpu.VMEM((2, B, SQ, GW), bf16),
            pltpu.VMEM((SQ, GW), bf16),
            pltpu.VMEM((B, SQ, D), f32),
            pltpu.VMEM((B, SQ, D), bf16),
            pltpu.SemaphoreType.DMA(()),
            pltpu.SemaphoreType.DMA((L,)),
            pltpu.SemaphoreType.DMA((L,)),
            pltpu.SemaphoreType.DMA((NG,)),
            pltpu.SemaphoreType.DMA((NG,)),
            pltpu.SemaphoreType.DMA((2,)),
        ],
        compiler_params=pltpu.CompilerParams(
            vmem_limit_bytes=48 * 1024 * 1024,
            disable_bounds_checks=True,
            disable_semaphore_checks=True,
        ),
    )(x, k_cache, v_cache, wq, wo)
```
